```python
import jax
import jax.numpy as jnp

def _softmax(x, axis=-1):
    return jax.nn.softmax(x, axis=axis)
def _gelu(x):
    return jax.nn.gelu(x, approximate=True)
def _silu(x):
    return jax.nn.silu(x)
def _sigmoid(x):
    return jax.nn.sigmoid(x)
def _layernorm(x, axis=-1, eps=1e-5):
    m = jnp.mean(x, axis=axis, keepdims=True)
    v = jnp.var(x, axis=axis, keepdims=True)
    return (x - m) / jnp.sqrt(v + eps)
def _scatter_add(tgt, idx, src, axis=0):
    return tgt.at[idx].add(src)
def _segment_sum(src, seg, n):
    return jax.ops.segment_sum(src, seg, n)
class _Rng:
    def __init__(self, key):
        self._k = key
    def _next(self):
        self._k, sub = jax.random.split(self._k)
        return sub
    def normal(self, shape):
        return jax.random.normal(self._next(), shape, dtype=jnp.bfloat16)
    def randint(self, lo, hi, shape):
        return jax.random.randint(self._next(), shape, lo, hi, dtype=jnp.int32)
    def uniform(self, shape, lo=0.0, hi=1.0):
        return jax.random.uniform(self._next(), shape, jnp.bfloat16, lo, hi)
    def permutation(self, n):
        return jax.random.permutation(self._next(), n)


kernel_name = 'standalone__fused_io_aware_attn__prompt'

def setup_inputs():
    _rng = _Rng(jax.random.key(int.from_bytes(__import__("os").urandom(4), "little")))
    _w = (lambda a: (lambda t: t.astype(jnp.bfloat16) if jnp.issubdtype(t.dtype, jnp.floating) else t)(jnp.asarray(a)))
    B, H, S = 2, 32, 2048
    Dh = max(1, 1024 // 32)
    return {
        "q": _w((lambda *s: _rng.normal(s) * 0.05)(B, H, S, Dh)),
        "k": _w((lambda *s: _rng.normal(s) * 0.05)(B, H, S, Dh)),
        "v": _w((lambda *s: _rng.normal(s) * 0.05)(B, H, S, Dh)),
    }

def reference(q, k, v):
    scale = q.shape[-1] ** -0.5
    s = jnp.einsum('bhqd,bhkd->bhqk', q, k) * scale
    p = _softmax(s, axis=-1)
    return jnp.einsum('bhqk,bhkd->bhqd', p, v)
```

```python
import functools

import jax
import jax.numpy as jnp
import numpy as np
from jax import lax
import jax.experimental.pallas as pl
import jax.experimental.pallas.tpu as pltpu

_L_MIN = 2.0 ** -16
_L_MAX = 2.0 ** 64
_ACC_MAX = 2.0 ** 126


def _fast_head(q_ref, k_ref, v_ref, o_ref, ks_ref, h, *, c, bk):
    d, s_len = q_ref.shape[1:]
    ks_ref[h] = k_ref[h].T
    q_t = (q_ref[h].astype(jnp.float32) * c).astype(jnp.bfloat16)
    acc = jnp.zeros((d, s_len), jnp.float32)
    l = jnp.zeros((8, s_len), jnp.float32)
    for j in range(s_len // bk):
        s = jnp.dot(ks_ref[h, j * bk:(j + 1) * bk, :], q_t,
                    preferred_element_type=jnp.float32)
        p = jnp.exp2(s)
        l = l + p.reshape(bk // 8, 8, s_len).sum(0)
        acc = acc + jnp.dot(v_ref[h, :, j * bk:(j + 1) * bk],
                            p.astype(jnp.bfloat16),
                            preferred_element_type=jnp.float32)
    ls = l.sum(0, keepdims=True)
    o_ref[h] = (acc / ls).astype(o_ref.dtype)
    ok = jnp.logical_and(ls >= _L_MIN, ls <= _L_MAX)
    ok = jnp.logical_and(ok, jnp.abs(acc) <= _ACC_MAX)
    return jnp.max(jnp.where(ok, 0.0, 1.0))


def _safe_head(q_ref, k_ref, v_ref, o_ref, ks_ref, h, *, scale, bq, bk):
    d, s_len = q_ref.shape[1:]

    def q_body(i, carry):
        q0 = pl.multiple_of(i * bq, bq)
        q_t = q_ref[h, :, pl.ds(q0, bq)]

        def k_body(j, state):
            m, l, acc = state
            k0 = pl.multiple_of(j * bk, bk)
            s = jnp.dot(ks_ref[h, pl.ds(k0, bk), :], q_t,
                        preferred_element_type=jnp.float32) * scale
            m_new = jnp.maximum(m, s.max(0, keepdims=True))
            alpha = jnp.exp(m - m_new)
            p = jnp.exp(s - m_new)
            l = alpha * l + p.sum(0, keepdims=True)
            acc = alpha * acc + jnp.dot(v_ref[h, :, pl.ds(k0, bk)],
                                        p.astype(jnp.bfloat16),
                                        preferred_element_type=jnp.float32)
            return m_new, l, acc

        init = (jnp.full((1, bq), -jnp.inf, jnp.float32),
                jnp.zeros((1, bq), jnp.float32),
                jnp.zeros((d, bq), jnp.float32))
        _, l, acc = lax.fori_loop(0, s_len // bk, k_body, init)
        o_ref[h, :, pl.ds(q0, bq)] = (acc / l).astype(o_ref.dtype)
        return carry

    lax.fori_loop(0, s_len // bq, q_body, 0)


def _kernel(q_ref, k_ref, v_ref, o_ref, ks_ref, *, scale, nh, bk):
    c = float(scale * np.log2(np.e))
    bad = [_fast_head(q_ref, k_ref, v_ref, o_ref, ks_ref, h, c=c, bk=bk)
           for h in range(nh)]
    any_bad = functools.reduce(jnp.maximum, bad)

    @pl.when(any_bad > 0.0)
    def _():
        def body(h, carry):
            _safe_head(q_ref, k_ref, v_ref, o_ref, ks_ref, h,
                       scale=scale, bq=256, bk=256)
            return carry
        lax.fori_loop(0, nh, body, 0)


@jax.jit
def pallas_standalone__fused_io_aware_attn__prompt_kernel(
    q: jax.Array,
    k: jax.Array,
    v: jax.Array,
):
    b, h, s, d = q.shape
    nh = 4
    scale = float(d ** -0.5)

    def t(x):
        return x.transpose(0, 1, 3, 2).reshape(b * h, d, s)

    spec = pl.BlockSpec((nh, d, s), lambda i: (i, 0, 0))
    out = pl.pallas_call(
        functools.partial(_kernel, scale=scale, nh=nh, bk=256),
        grid=(b * h // nh,),
        in_specs=[spec] * 3,
        out_specs=spec,
        out_shape=jax.ShapeDtypeStruct((b * h, d, s), q.dtype),
        scratch_shapes=[pltpu.VMEM((nh, s, d), jnp.bfloat16)],
        compiler_params=pltpu.CompilerParams(
            dimension_semantics=("parallel",),
            vmem_limit_bytes=100 * 1024 * 1024),
    )(t(q), t(k), t(v))
    return out.reshape(b, h, d, s).transpose(0, 1, 3, 2)
```

```python
import functools

import jax
import jax.numpy as jnp
import numpy as np
from jax import lax
import jax.experimental.pallas as pl
import jax.experimental.pallas.tpu as pltpu

_L_MIN = 2.0 ** -16
_L_MAX = 2.0 ** 64
_ACC_MAX = 2.0 ** 126


def _fast_head(q_ref, k_ref, v_ref, o_ref, ks_ref, h, *, c, bk):
    d, s_len = q_ref.shape[1:]
    ks_ref[h] = k_ref[h].T
    q_t = (q_ref[h].astype(jnp.float32) * c).astype(jnp.bfloat16)
    acc = jnp.zeros((d, s_len), jnp.float32)
    l = jnp.zeros((8, s_len), jnp.float32)
    for j in range(s_len // bk):
        s = jnp.dot(ks_ref[h, j * bk:(j + 1) * bk, :], q_t,
                    preferred_element_type=jnp.float32)
        p = jnp.exp2(s)
        l = l + p.reshape(bk // 8, 8, s_len).sum(0)
        acc = acc + jnp.dot(v_ref[h, :, j * bk:(j + 1) * bk],
                            p.astype(jnp.bfloat16),
                            preferred_element_type=jnp.float32)
    ls = l.sum(0, keepdims=True)
    o_ref[h] = (acc / ls).astype(o_ref.dtype)
    mag = jnp.abs(acc).reshape(d // 8, 8, s_len // 128, 128).sum((0, 2))
    ok = jnp.logical_and(ls >= _L_MIN, ls <= _L_MAX)
    low = jnp.where(ok, 0.0, 1.0)
    return jnp.where(mag <= _ACC_MAX, 0.0, 1.0), low


def _safe_head(q_ref, k_ref, v_ref, o_ref, ks_ref, h, *, scale, bq, bk):
    d, s_len = q_ref.shape[1:]

    def q_body(i, carry):
        q0 = pl.multiple_of(i * bq, bq)
        q_t = q_ref[h, :, pl.ds(q0, bq)]

        def k_body(j, state):
            m, l, acc = state
            k0 = pl.multiple_of(j * bk, bk)
            s = jnp.dot(ks_ref[h, pl.ds(k0, bk), :], q_t,
                        preferred_element_type=jnp.float32) * scale
            m_new = jnp.maximum(m, s.max(0, keepdims=True))
            alpha = jnp.exp(m - m_new)
            p = jnp.exp(s - m_new)
            l = alpha * l + p.sum(0, keepdims=True)
            acc = alpha * acc + jnp.dot(v_ref[h, :, pl.ds(k0, bk)],
                                        p.astype(jnp.bfloat16),
                                        preferred_element_type=jnp.float32)
            return m_new, l, acc

        init = (jnp.full((1, bq), -jnp.inf, jnp.float32),
                jnp.zeros((1, bq), jnp.float32),
                jnp.zeros((d, bq), jnp.float32))
        _, l, acc = lax.fori_loop(0, s_len // bk, k_body, init)
        o_ref[h, :, pl.ds(q0, bq)] = (acc / l).astype(o_ref.dtype)
        return carry

    lax.fori_loop(0, s_len // bq, q_body, 0)


def _kernel(q_ref, k_ref, v_ref, o_ref, ks_ref, *, scale, nh, bk):
    c = float(scale * np.log2(np.e))
    bad = [_fast_head(q_ref, k_ref, v_ref, o_ref, ks_ref, h, c=c, bk=bk)
           for h in range(nh)]
    any_bad = jnp.maximum(
        jnp.max(functools.reduce(jnp.maximum, [b[0] for b in bad])),
        jnp.max(functools.reduce(jnp.maximum, [b[1] for b in bad])))

    @pl.when(any_bad > 0.0)
    def _():
        def body(h, carry):
            _safe_head(q_ref, k_ref, v_ref, o_ref, ks_ref, h,
                       scale=scale, bq=256, bk=256)
            return carry
        lax.fori_loop(0, nh, body, 0)


@jax.jit
def pallas_standalone__fused_io_aware_attn__prompt_kernel(
    q: jax.Array,
    k: jax.Array,
    v: jax.Array,
):
    b, h, s, d = q.shape
    nh = 4
    scale = float(d ** -0.5)

    def t(x):
        return x.transpose(0, 1, 3, 2).reshape(b * h, d, s)

    spec = pl.BlockSpec((nh, d, s), lambda i: (i, 0, 0))
    out = pl.pallas_call(
        functools.partial(_kernel, scale=scale, nh=nh, bk=256),
        grid=(b * h // nh,),
        in_specs=[spec] * 3,
        out_specs=spec,
        out_shape=jax.ShapeDtypeStruct((b * h, d, s), q.dtype),
        scratch_shapes=[pltpu.VMEM((nh, s, d), jnp.bfloat16)],
        compiler_params=pltpu.CompilerParams(
            dimension_semantics=("parallel",),
            vmem_limit_bytes=100 * 1024 * 1024),
    )(t(q), t(k), t(v))
    return out.reshape(b, h, d, s).transpose(0, 1, 3, 2)
```

```python
import functools

import jax
import jax.numpy as jnp
import numpy as np
from jax import lax
import jax.experimental.pallas as pl
import jax.experimental.pallas.tpu as pltpu

_L_MIN = 2.0 ** -16
_L_MAX = 2.0 ** 64
_ACC_MAX = 2.0 ** 126


def _fast_heads(q_ref, k_ref, v_ref, o_ref, ks_ref, *, c, bq, bk):
    nh, d, s_len = q_ref.shape
    nj = s_len // bk
    steps = [(h, i, j) for h in range(nh) for i in range(s_len // bq)
             for j in range(nj)]
    q_t = {}

    def prepare(h):
        ks_ref[h] = k_ref[h].T
        for i in range(s_len // bq):
            qs = q_ref[h, :, i * bq:(i + 1) * bq].astype(jnp.float32) * c
            q_t[h, i] = qs.astype(jnp.bfloat16)

    def scores(h, i, j):
        return jnp.dot(ks_ref[h, j * bk:(j + 1) * bk, :], q_t[h, i],
                       preferred_element_type=jnp.float32)

    prepare(0)
    s_next = scores(*steps[0])
    bad = jnp.zeros((8, 128), jnp.float32)
    low = jnp.zeros((1, bq), jnp.float32)
    for n, (h, i, j) in enumerate(steps):
        if j == 0:
            acc = jnp.zeros((d, bq), jnp.float32)
            l = jnp.zeros((8, bq), jnp.float32)
        if n % (len(steps) // nh) == 2 and h + 1 < nh:
            prepare(h + 1)
        s = s_next
        if n + 1 < len(steps):
            s_next = scores(*steps[n + 1])
        p = jnp.exp2(s)
        l = l + p.reshape(bk // 8, 8, bq).sum(0)
        acc = acc + jnp.dot(v_ref[h, :, j * bk:(j + 1) * bk],
                            p.astype(jnp.bfloat16),
                            preferred_element_type=jnp.float32)
        if j == nj - 1:
            ls = l.sum(0, keepdims=True)
            o_ref[h, :, i * bq:(i + 1) * bq] = (acc / ls).astype(o_ref.dtype)
            mag = jnp.abs(acc).reshape(d // 8, 8, bq // 128, 128).sum((0, 2))
            bad = jnp.where(mag <= _ACC_MAX, bad, 1.0)
            ok = jnp.logical_and(ls >= _L_MIN, ls <= _L_MAX)
            low = jnp.where(ok, low, 1.0)
    return jnp.maximum(jnp.max(bad), jnp.max(low))


def _safe_head(q_ref, k_ref, v_ref, o_ref, ks_ref, h, *, scale, bq, bk):
    d, s_len = q_ref.shape[1:]

    def q_body(i, carry):
        q0 = pl.multiple_of(i * bq, bq)
        q_t = q_ref[h, :, pl.ds(q0, bq)]

        def k_body(j, state):
            m, l, acc = state
            k0 = pl.multiple_of(j * bk, bk)
            s = jnp.dot(ks_ref[h, pl.ds(k0, bk), :], q_t,
                        preferred_element_type=jnp.float32) * scale
            m_new = jnp.maximum(m, s.max(0, keepdims=True))
            alpha = jnp.exp(m - m_new)
            p = jnp.exp(s - m_new)
            l = alpha * l + p.sum(0, keepdims=True)
            acc = alpha * acc + jnp.dot(v_ref[h, :, pl.ds(k0, bk)],
                                        p.astype(jnp.bfloat16),
                                        preferred_element_type=jnp.float32)
            return m_new, l, acc

        init = (jnp.full((1, bq), -jnp.inf, jnp.float32),
                jnp.zeros((1, bq), jnp.float32),
                jnp.zeros((d, bq), jnp.float32))
        _, l, acc = lax.fori_loop(0, s_len // bk, k_body, init)
        o_ref[h, :, pl.ds(q0, bq)] = (acc / l).astype(o_ref.dtype)
        return carry

    lax.fori_loop(0, s_len // bq, q_body, 0)


def _kernel(q_ref, k_ref, v_ref, o_ref, ks_ref, *, scale, nh, bk):
    c = float(scale * np.log2(np.e))
    any_bad = _fast_heads(q_ref, k_ref, v_ref, o_ref, ks_ref, c=c, bq=2048, bk=bk)

    @pl.when(any_bad > 0.0)
    def _():
        def body(h, carry):
            _safe_head(q_ref, k_ref, v_ref, o_ref, ks_ref, h,
                       scale=scale, bq=256, bk=256)
            return carry
        lax.fori_loop(0, nh, body, 0)


@jax.jit
def pallas_standalone__fused_io_aware_attn__prompt_kernel(
    q: jax.Array,
    k: jax.Array,
    v: jax.Array,
):
    b, h, s, d = q.shape
    nh = 4
    scale = float(d ** -0.5)

    def t(x):
        return x.transpose(0, 1, 3, 2).reshape(b * h, d, s)

    spec = pl.BlockSpec((nh, d, s), lambda i: (i, 0, 0))
    out = pl.pallas_call(
        functools.partial(_kernel, scale=scale, nh=nh, bk=256),
        grid=(b * h // nh,),
        in_specs=[spec] * 3,
        out_specs=spec,
        out_shape=jax.ShapeDtypeStruct((b * h, d, s), q.dtype),
        scratch_shapes=[pltpu.VMEM((nh, s, d), jnp.bfloat16)],
        compiler_params=pltpu.CompilerParams(
            dimension_semantics=("parallel",),
            vmem_limit_bytes=100 * 1024 * 1024),
    )(t(q), t(k), t(v))
    return out.reshape(b, h, d, s).transpose(0, 1, 3, 2)
```
